```python
import os as _os
_os.environ.setdefault('JAX_PLATFORMS', 'cpu')
import jax
import jax.numpy as jnp

def _softmax(x, axis=-1):
    return jax.nn.softmax(x, axis=axis)

def _gelu(x):
    return jax.nn.gelu(x, approximate=True)

def _silu(x):
    return jax.nn.silu(x)

def _sigmoid(x):
    return jax.nn.sigmoid(x)

def _layernorm(x, axis=-1, eps=1e-05):
    m = jnp.mean(x, axis=axis, keepdims=True)
    v = jnp.var(x, axis=axis, keepdims=True)
    return (x - m) / jnp.sqrt(v + eps)

def _scatter_add(tgt, idx, src, axis=0):
    return tgt.at[idx].add(src)

def _segment_sum(src, seg, n):
    return jax.ops.segment_sum(src, seg, n)

class _Rng:

    def __init__(self, key):
        self._k = key

    def _next(self):
        self._k, sub = jax.random.split(self._k)
        return sub

    def normal(self, shape):
        return jax.random.normal(self._next(), shape, dtype=jnp.bfloat16)

    def randint(self, lo, hi, shape):
        return jax.random.randint(self._next(), shape, lo, hi, dtype=jnp.int32)

    def uniform(self, shape, lo=0.0, hi=1.0):
        return jax.random.uniform(self._next(), shape, jnp.bfloat16, lo, hi)

    def permutation(self, n):
        return jax.random.permutation(self._next(), n)
kernel_name = 'parallel_sum__memory_aug_recurrent_mem_tr__dense_activation_silu__prompt'

def setup_inputs():
    _rng = _Rng(jax.random.key(int.from_bytes(__import__("os").urandom(4), "little")))
    _w = lambda a: (lambda t: t.astype(jnp.bfloat16) if jnp.issubdtype(t.dtype, jnp.floating) else t)(jnp.asarray(a))

    def _A_setup():
        B, S, Dm = (1, 2048, 448)
        H, Dh = (16, 256)
        M, seg = (8, 32)
        seg = min(seg, S)
        S = S // seg * seg
        return {'x': _w((lambda *s: _rng.normal(s) * 0.05)(B, S, Dm)), 'mem0': _w((lambda *s: _rng.normal(s) * 0.2)(B, M, Dm)), 'Wq': _w((lambda *s: _rng.normal(s) * 0.8)(Dm, H, Dh) * Dm ** (-0.5)), 'Wk': _w((lambda *s: _rng.normal(s) * 0.8)(Dm, H, Dh) * Dm ** (-0.5)), 'Wv': _w((lambda *s: _rng.normal(s) * 0.2)(Dm, H, Dh) * Dm ** (-0.5)), 'Wo': _w((lambda *s: _rng.normal(s) * 0.2)(H, Dh, Dm) * (H * Dh) ** (-0.5)), 'seg_len': seg}
    _A_in = _A_setup()

    def _B_setup():
        B, S, D, F = (1, 2048, 448, 1792)
        return {'x': _w((lambda *s: _rng.normal(s) * 0.05)(B, S, D)), 'w1': _w((lambda *s: _rng.normal(s) * 0.05)(D, F) * D ** (-0.5)), 'w2': _w((lambda *s: _rng.normal(s) * 0.05)(F, D) * F ** (-0.5))}
    _B_in = _B_setup()
    return {'A_x': _A_in['x'], 'A_mem0': _A_in['mem0'], 'A_Wq': _A_in['Wq'], 'A_Wk': _A_in['Wk'], 'A_Wv': _A_in['Wv'], 'A_Wo': _A_in['Wo'], 'A_seg_len': _A_in['seg_len'], 'B_x': _B_in['x'], 'B_w1': _B_in['w1'], 'B_w2': _B_in['w2']}

def reference(A_x, A_mem0, A_Wq, A_Wk, A_Wv, A_Wo, A_seg_len, B_x, B_w1, B_w2):

    def _A_ref(x, mem0, Wq, Wk, Wv, Wo, seg_len):
        B, S, Dm = x.shape
        H, Dh = (Wq.shape[1], Wq.shape[2])
        M = mem0.shape[1]
        scale = Dh ** (-0.5)
        n_seg = S // seg_len
        L = M + seg_len
        idx = jnp.arange(L)
        mask = (idx[:, None] < M) | (idx[:, None] >= idx[None, :])
        mem = mem0
        outs = []
        for s in range(n_seg):
            xs = x[:, s * seg_len:(s + 1) * seg_len, :].copy()
            h = jnp.concatenate([mem, xs], axis=1)
            q = jnp.einsum('btd,dhe->bhte', h, Wq)
            k = jnp.einsum('btd,dhe->bhte', h, Wk)
            v = jnp.einsum('btd,dhe->bhte', h, Wv)
            scores = jnp.einsum('bhqe,bhke->bhqk', q, k) * scale
            scores = jnp.where(mask[None, None], scores, -1000000000.0)
            p = _softmax(scores, axis=-1)
            o = jnp.einsum('bhqk,bhke->bhqe', p, v)
            o = jnp.einsum('bhte,hed->btd', o, Wo)
            mem = o[:, :M, :].copy()
            outs.append(o[:, M:, :])
        return jnp.concatenate(outs, axis=1)

    def _B_ref(x, w1, w2):
        h = jnp.einsum('bsd,df->bsf', x, w1)
        h = _silu(h)
        out = jnp.einsum('bsf,fd->bsd', h, w2)
        return out
    x = A_x
    xn = _layernorm(x, axis=-1)
    return x + _A_ref(xn, A_mem0, A_Wq, A_Wk, A_Wv, A_Wo, A_seg_len) + _B_ref(xn, B_w1, B_w2)
```

```python
import jax
import jax.numpy as jnp
from jax.experimental import pallas as pl
from jax.experimental.pallas import tpu as pltpu

D = 448
DP = 512
H = 16
E = 256
F = 1792
S = 2048
SEG = 32
NSEG = S // SEG
NG = NSEG // 4
NGRUN = NG
PARTS = (512, 512, 512, 256)
POFF = tuple(sum(PARTS[:k]) for k in range(4))
GSPLIT = 2
ORDER = "T0 T1 T2 T3 Y0 S0 S1 S2 S3 S4 Y1 Y2 Y3 F P G O"
u32 = jnp.uint32
bf16 = jnp.bfloat16
f32 = jnp.float32
i32 = jnp.int32


def _bf(x):
    return pltpu.bitcast(x, bf16)


def _pk(x):
    return pltpu.bitcast(x.astype(bf16), u32)


def _T(x):
    return _bf(pltpu.bitcast(x.T, u32))


def _dot(a, b):
    return jnp.dot(a, b, preferred_element_type=f32)


def _dotm(a, b):
    return jax.lax.dot_general(a, b, (((1,), (0,)), ((), ())), preferred_element_type=f32)


def _dot_ntm(a, b):
    return jax.lax.dot_general(a, b, (((1,), (1,)), ((), ())), preferred_element_type=f32)


def _dot_nt(a, b):
    return jax.lax.dot_general(a, b, (((1,), (1,)), ((), ())), preferred_element_type=f32)


NSEM = 16


def kernel(x_h, mem_h, wq_h, wk_h, wv_h, wo_h, w1_h, w2_h, o_h,
           xv, memv, wqv, wkv, wvv, wov, w1v, w2v,
           wc, w1t, xnt, hts, ots, xn32, stq, stk, kde, msk, ob, rb, sem, osem):
    def cp(src, dst, k):
        return pltpu.make_async_copy(src, dst, sem.at[k])

    QR = D * H // 4
    cp_m = cp(mem_h, memv, 0)
    cp_k = cp(wk_h, wkv, 1)
    cp_q = [cp(wq_h.at[pl.ds(QR * c, QR)], wqv.at[pl.ds(QR * c, QR)], 2 + c) for c in range(4)]
    cp_o = cp(wo_h, wov, 6)
    cp_v = [cp(wv_h.at[pl.ds(QR * c, QR)], wvv.at[pl.ds(QR * c, QR)], 7 + c) for c in range(4)]
    cp_x = [cp(x_h.at[:, pl.ds(1024 * c, 1024)], xv.at[:, pl.ds(1024 * c, 1024)], 11 + c) for c in range(2)]
    cp_1 = [cp(w1_h.at[:, pl.ds(896 * c, 896)], w1v.at[:, pl.ds(896 * c, 896)], 13 + c) for c in range(2)]
    cp_2 = cp(w2_h, w2v, 15)
    for c_ in [cp_m, cp_k] + cp_q + [cp_o] + cp_v + cp_x + cp_1 + [cp_2]:
        c_.start()

    k_i = jax.lax.broadcasted_iota(i32, (40, 128), 0)
    l_i = jax.lax.broadcasted_iota(i32, (40, 128), 1)
    q_i = l_i % 32
    msk[0] = ((q_i < 8) | (k_i <= q_i)).astype(i32)
    msk[1] = (k_i <= 32 + l_i % 8).astype(i32)
    wc[:, 0:32, :] = jnp.zeros((4, 32, 3584), u32)

    def ln_block(g):
        xb = xv[:, g * 128:(g + 1) * 128].astype(f32)
        m = jnp.mean(xb, axis=0, keepdims=True)
        xc = xb - m
        v = jnp.mean(xc * xc, axis=0, keepdims=True)
        xn = xc * jax.lax.rsqrt(v + 1e-5)
        xn = jnp.concatenate([jnp.zeros((64, 128), f32), xn], axis=0).astype(bf16)
        xnt[:, g * 128:(g + 1) * 128] = xn
        xn32[g * 128:(g + 1) * 128, :] = xn.T.astype(f32)

    def stage(src, dst, d0, nd):
        for r in range(0, nd, 56):
            u = pltpu.bitcast(src[16 * (d0 + r):16 * (d0 + r + 56), :], u32)
            for dd in range(56):
                pos = ((r + dd) % 2) * (nd // 2) + (r + dd) // 2
                for half in range(2):
                    dst[half, pl.ds(pos, 8, stride=nd + 2), :] = u[8 * dd:8 * dd + 8, 128 * half:128 * half + 128]

    def pair_rows(st, j, nd):
        return jnp.concatenate([st[half, pl.ds(j * (nd + 2), nd), :] for half in range(2)], axis=1)

    def lhs_heads(st, j, nd):
        u = pair_rows(st, j, nd)
        return pltpu.bitcast(u << 16, f32), pltpu.bitcast(u & u32(0xffff0000), f32)

    def pack_rows(r):
        n = r.shape[0] // 2
        return pltpu.bitcast(pltpu.pack_elementwise([r[:n], r[n:]], packed_dtype=bf16), u32)

    def w1_block(c):
        blk = w1v[:, c * 128:(c + 1) * 128]
        blk = jnp.concatenate([jnp.zeros((64, 128), bf16), blk], axis=0)
        w1t[c * 64:(c + 1) * 64, :] = pltpu.bitcast(blk.T, u32)

    KS = 258

    def make_kde():
        for half in range(2):
            for h in range(H):
                kde[half, pl.ds(h * KS, 32), :] = jnp.zeros((32, 128), u32)
        for r in range(0, D, 56):
            u = pltpu.bitcast(wkv[16 * r:16 * (r + 56), :], u32)
            for s_ in range(28):
                a, b_ = u[16 * s_:16 * s_ + 8], u[16 * s_ + 8:16 * s_ + 16]
                lo = (a & u32(0xffff)) | (b_ << 16)
                hi = (a >> 16) | (b_ & u32(0xffff0000))
                row = 32 + r // 2 + s_
                for half in range(2):
                    kde[half, pl.ds(row, 8, stride=2 * KS), :] = lo[:, 128 * half:128 * half + 128]
                    kde[half, pl.ds(row + KS, 8, stride=2 * KS), :] = hi[:, 128 * half:128 * half + 128]

    def kde_head(h):
        return _bf(jnp.concatenate([kde[half, pl.ds(h * KS, 256), :] for half in range(2)], axis=1))

    def chunk_ref(st, c):
        return st.at[:, pl.ds(c * 8 * 114, 8 * 114), :]

    cp_k.wait()
    make_kde()
    cp_q[0].wait()
    stage(wqv, chunk_ref(stq, 0), 0, 112)
    for c in range(4):
        for j in range(8):
            qs = lhs_heads(chunk_ref(stq, c), j, 112)
            for b in range(2):
                h = 2 * j + b
                a_sh = pack_rows(_dot_ntm(qs[b], kde_head(h)))
                col = (h % 4) * 896 + 384
                wc[h // 4, 32 + 56 * c:32 + 56 * (c + 1), col:col + 512] = a_sh
            if j == 4:
                if c < 3:
                    cp_q[c + 1].wait()
                    stage(wqv, chunk_ref(stq, c + 1), 112 * (c + 1), 112)
                else:
                    cp_v[0].wait()
                    stage(wvv, chunk_ref(stk, 0), 0, 112)
                    cp_o.wait()

    for c in range(4):
        for j in range(8):
            vs = lhs_heads(chunk_ref(stk, c), j, 112)
            for b in range(2):
                h = 2 * j + b
                wo = jnp.concatenate([wov[h], jnp.zeros((64, E), bf16)], axis=0)
                bm = pack_rows(_dot_ntm(vs[b], wo))
                rows = slice(32 + 56 * c, 32 + 56 * (c + 1))
                col = (h % 4) * 896
                wc[h // 4, rows, col:col + 384] = bm[:, :384]
                wc[h // 4, rows, col + 384:col + 512] = wc[h // 4, rows, col + 384:col + 512] | bm[:, 384:]
            if j == 4 and c < 3:
                cp_v[c + 1].wait()
                stage(wvv, chunk_ref(stk, c + 1), 112 * (c + 1), 112)
            if c >= 2:
                if j == 0:
                    cp_x[c - 2].wait()
                ln_block(8 * (c - 2) + j)
            if c == 3:
                if j == 2:
                    cp_1[0].wait()
                if j == 5:
                    cp_1[1].wait()
                for blk in {2: (0, 1, 2), 3: (3, 4, 5), 4: (6,), 5: (7, 8, 9), 6: (10, 11), 7: (12, 13)}.get(j, ()):
                    w1_block(blk)

    hts[...] = jnp.zeros(hts.shape, hts.dtype)
    ots[...] = jnp.zeros(ots.shape, ots.dtype)
    cp_2.wait()

    cp_m.wait()
    mem0 = memv[...].astype(f32)
    mem0 = jnp.concatenate([jnp.zeros((8, 64), f32), mem0], axis=1)

    lane = jax.lax.broadcasted_iota(i32, (8, 128), 1)
    lane32 = jax.lax.broadcasted_iota(i32, (32, 128), 1)

    def softmax(sc, mask):
        sc = jnp.where(mask, sc * (E ** -0.5), -1e9)
        mx = jnp.max(sc, axis=0, keepdims=True)
        e = jnp.exp(sc - mx)
        l = jnp.sum(e, axis=0, keepdims=True)
        return e * (1.0 / l)

    def seg_step(g, i, mem_sh, ffn, hook=None):
        xr = xn32[pl.ds(pl.multiple_of(g * 128 + i * 32, 32), 32), :]
        h40 = jnp.concatenate([mem_sh, xr], axis=0)

        def wcol(h, lo, hi):
            return _bf(wc[h // 4, :, (h % 4) * 896 + lo:(h % 4) * 896 + hi])

        m0 = msk[0] != 0
        m1 = msk[1] != 0
        T = [None] * H
        Y = [None] * H
        P = [None] * 5
        box = {}
        hprev = hts[...] if i == 0 else ffn['h']

        def sdot(tb):
            return _dotm(h40, _T(tb))

        def do(op):
            kind, a = op[0], int(op[1:], 16) if len(op) > 1 else 0
            if kind == 'T':
                for h in range(4 * a, 4 * a + 4):
                    T[h] = _dotm(h40, wcol(h, 384, 896))
            elif kind == 'Y':
                for h in range(4 * a, 4 * a + 4):
                    Y[h] = jnp.concatenate([_dotm(h40, wcol(h, 0, 384)), T[h][:, :128]], axis=1)
            elif kind == 'S':
                if a < 4:
                    tc = jnp.concatenate([T[4 * a + b][0:32] for b in range(4)], axis=0).astype(bf16)
                    P[a] = softmax(sdot(tc), m0)
                else:
                    tc = jnp.concatenate([T[h][32:40] for h in range(H)], axis=0).astype(bf16)
                    P[4] = softmax(sdot(tc), m1)
            elif kind == 'F':
                f0 = POFF[i]
                hpre = _dot(_bf(w1t[f0 // 2:(f0 + PARTS[i]) // 2, :]), xnt[:, pl.ds(pl.multiple_of(g * 128, 128), 128)])
                ffn['h'] = (hpre * jax.nn.sigmoid(hpre)).astype(bf16)
            elif kind == 'G':
                p = (i - 1) % 4
                f0 = POFF[p]
                rs = D // GSPLIT
                o = jnp.concatenate([_dot(w2v[r * rs:(r + 1) * rs, f0:f0 + PARTS[p]], hprev) for r in range(GSPLIT)], axis=0)
                ffn['o'] = (ots[...] if i == 0 else ffn['o']) + o if i != 1 else o
            elif kind == 'P':
                box['R'] = do_py()

        def do_py():
            m1t = jnp.concatenate([P[a][0:32] for a in range(4)], axis=0).T
            m3 = jnp.concatenate([jnp.where(lane // 32 == b, P[a][32:40], 0.0)
                                  for a in range(4) for b in range(4)], axis=0)
            m3t = m3.T
            m3t = (m3t[0:32] + m3t[32:64]) + (m3t[64:96] + m3t[96:128])
            m4 = jnp.concatenate([jnp.where(lane32 // 32 == a, P[4][0:32], 0.0) for a in range(4)], axis=0)
            m4t = m4.T
            m5 = jnp.concatenate([jnp.where(lane // 8 == hh, P[4][32:40], 0.0) for hh in range(16)], axis=0)
            m5t = m5.T
            w = m5t[0:8]
            for r in range(1, 16):
                w = w + m5t[8 * r:8 * r + 8]
            pcat = []
            for gg in range(4):
                third = m4t[8 * gg:8 * gg + 8]
                for a in range(1, 4):
                    third = third + m4t[8 * (4 * a + gg):8 * (4 * a + gg) + 8]
                pcat.append(jnp.concatenate([m1t[32 * gg:32 * gg + 32], third], axis=0))
            pcat.append(jnp.concatenate([m3t, w], axis=0))
            pcat = jnp.concatenate(pcat, axis=1)
            ycat = [jnp.concatenate([Y[4 * a + gg][0:32] for a in range(4)], axis=0).astype(bf16) for gg in range(4)]
            ycat.append(jnp.concatenate([Y[h][32:40] for h in range(H)], axis=0).astype(bf16))
            ycat = jnp.concatenate(ycat, axis=0)
            return _dotm(pcat, ycat)

        for op in ORDER.split():
            if op == 'O':
                if hook is not None:
                    hook()
            else:
                do(op)
        R = box['R']
        res = R[8:40]
        mem_next = jnp.concatenate([jnp.zeros((8, 64), f32), R[0:8, :D]], axis=1)
        return mem_next, res

    def out_copy(g):
        cols = pl.ds(pl.multiple_of(g * 128, 128), 128)
        return pltpu.make_async_copy(ob.at[:, cols], o_h.at[:, cols], osem.at[0])

    def flush(g, ffn_t):
        cols = pl.ds(pl.multiple_of(g * 128, 128), 128)
        rt = rb[...].T
        ob[:, cols] = (xv[:, cols].astype(f32) + (rt[:D] + ffn_t)).astype(ob.dtype)

    rb[...] = jnp.zeros(rb.shape, rb.dtype)

    def body(g, mem_sh):
        gp = jnp.maximum(g - 1, 0)
        ffn = {}
        for i in range(4):
            hook = (lambda: flush(gp, ffn['o'])) if i == 0 else None
            mem_sh, r = seg_step(g, i, mem_sh, ffn, hook)
            rb[i * 32:(i + 1) * 32, :] = r
        hts[...] = ffn['h']
        ots[...] = ffn['o']

        @pl.when(g > 0)
        def _():
            out_copy(g - 1).start()
        return mem_sh

    jax.lax.fori_loop(0, NGRUN, body, mem0)
    rs = D // GSPLIT
    f0 = POFF[3]
    o = jnp.concatenate([_dot(w2v[r * rs:(r + 1) * rs, f0:f0 + PARTS[3]], hts[...]) for r in range(GSPLIT)], axis=0)
    flush(NGRUN - 1, ots[...] + o)
    out_copy(NGRUN - 1).start()
    for g_ in range(NGRUN):
        out_copy(g_).wait()


@jax.jit
def pallas_parallel_sum__memory_aug_recurrent_mem_tr__dense_activation_silu__prompt_kernel(
    A_x,
    A_mem0,
    A_Wq,
    A_Wk,
    A_Wv,
    A_Wo,
    A_seg_len,
    B_x,
    B_w1,
    B_w2,
):
    dt = A_x.dtype
    any_spec = pl.BlockSpec(memory_space=pl.ANY)
    out = pl.pallas_call(
        kernel,
        out_shape=jax.ShapeDtypeStruct((D, S), dt),
        in_specs=[any_spec] * 8,
        out_specs=any_spec,
        scratch_shapes=[
            pltpu.VMEM((D, S), dt),
            pltpu.VMEM((8, D), dt),
            pltpu.VMEM((D * H, E), dt),
            pltpu.VMEM((D * H, E), dt),
            pltpu.VMEM((D * H, E), dt),
            pltpu.VMEM((H, D, E), dt),
            pltpu.VMEM((D, F), dt),
            pltpu.VMEM((D, F), dt),
            pltpu.VMEM((4, 256, 3584), u32),
            pltpu.VMEM((F // 2, DP), u32),
            pltpu.VMEM((DP, S), dt),
            pltpu.VMEM((PARTS[3], 128), dt),
            pltpu.VMEM((D, 128), f32),
            pltpu.VMEM((S, DP), f32),
            pltpu.VMEM((2, 3648, 128), u32),
            pltpu.VMEM((2, 3648, 128), u32),
            pltpu.VMEM((2, H * 258, 128), u32),
            pltpu.VMEM((2, 40, 128), i32),
            pltpu.VMEM((D, S), dt),
            pltpu.VMEM((128, DP), f32),
            pltpu.SemaphoreType.DMA((NSEM,)),
            pltpu.SemaphoreType.DMA((1,)),
        ],
        compiler_params=pltpu.CompilerParams(vmem_limit_bytes=110 * 1024 * 1024),
    )(A_x.reshape(S, D).T, A_mem0.reshape(8, D), A_Wq.reshape(D * H, E), A_Wk.reshape(D * H, E),
      A_Wv.reshape(D * H, E), jnp.transpose(A_Wo, (0, 2, 1)), B_w1, B_w2.T)
    return out.T.reshape(1, S, D)
```

```python
import jax
import jax.numpy as jnp
from jax.experimental import pallas as pl
from jax.experimental.pallas import tpu as pltpu

D = 448
DP = 512
H = 16
E = 256
F = 1792
S = 2048
SEG = 32
NSEG = S // SEG
NG = NSEG // 4
NGRUN = NG
PARTS = (512, 384, 512, 384)
POFF = tuple(sum(PARTS[:k]) for k in range(len(PARTS)))
FSCHED = ("F0,F1", "F2,G0", "G1,F3", "G2,G3")
LSTEP = 3
MIDJ = 4
GSPLIT = 2
ORDER = "T0 O T1 T2 T3 Y0 S0 S1 S2 S3 S4 Y1 Y2 Y3 a L P b"
u32 = jnp.uint32
bf16 = jnp.bfloat16
f32 = jnp.float32
i32 = jnp.int32


def _bf(x):
    return pltpu.bitcast(x, bf16)


def _pk(x):
    return pltpu.bitcast(x.astype(bf16), u32)


def _T(x):
    return _bf(pltpu.bitcast(x.T, u32))


def _dot(a, b):
    return jnp.dot(a, b, preferred_element_type=f32)


def _dotm(a, b):
    return jax.lax.dot_general(a, b, (((1,), (0,)), ((), ())), preferred_element_type=f32)


def _dot_ntm(a, b):
    return jax.lax.dot_general(a, b, (((1,), (1,)), ((), ())), preferred_element_type=f32)


def _dot_nt(a, b):
    return jax.lax.dot_general(a, b, (((1,), (1,)), ((), ())), preferred_element_type=f32)


NSEM = 22


def kernel(x_h, mem_h, wq_h, wk_h, wv_h, wo_h, w1_h, w2_h, o_h,
           xv, memv, wqv, wkv, wvv, wov, w1v, w2v,
           wc, w1t, xnt, ots, xn32, stq, stk, kde, msk, ob, rb, sem, osem):
    def cp(src, dst, k):
        return pltpu.make_async_copy(src, dst, sem.at[k])

    QR = D * H // 4
    KR = (0, 64, 192, 320, 448)
    cp_m = cp(mem_h, memv, 0)
    cp_v = [cp(wv_h.at[pl.ds(QR * c, QR)], wvv.at[pl.ds(QR * c, QR)], 1 + c) for c in range(4)]
    cp_o = [cp(wo_h.at[pl.ds(4 * g, 4)], wov.at[pl.ds(4 * g, 4)], 5 + g) for g in range(4)]
    cp_q = [cp(wq_h.at[pl.ds(QR * c, QR)], wqv.at[pl.ds(QR * c, QR)], 9 + c) for c in range(4)]
    cp_k = [cp(wk_h.at[pl.ds(16 * KR[t], 16 * (KR[t + 1] - KR[t]))],
               wkv.at[pl.ds(16 * KR[t], 16 * (KR[t + 1] - KR[t]))], 13 + t) for t in range(4)]
    cp_x = [cp(x_h.at[:, pl.ds(0, 256)], xv.at[:, pl.ds(0, 256)], 17),
            cp(x_h.at[:, pl.ds(256, S - 256)], xv.at[:, pl.ds(256, S - 256)], 18)]
    cp_1 = [cp(w1_h.at[:, pl.ds(896 * c, 896)], w1v.at[:, pl.ds(896 * c, 896)], 19 + c) for c in range(2)]
    cp_2 = cp(w2_h, w2v, 21)
    order = [cp_m]
    for c in range(4):
        order += [cp_v[c], cp_o[c]]
    order += [cp_q[0], cp_k[0], cp_k[1], cp_q[1], cp_k[2], cp_q[2], cp_k[3], cp_q[3], cp_x[0], cp_1[0], cp_1[1],
              cp_2, cp_x[1]]
    for c_ in order:
        c_.start()

    k_i = jax.lax.broadcasted_iota(i32, (40, 128), 0)
    l_i = jax.lax.broadcasted_iota(i32, (40, 128), 1)
    q_i = l_i % 32
    msk[0] = ((q_i < 8) | (k_i <= q_i)).astype(i32)
    msk[1] = (k_i <= 32 + l_i % 8).astype(i32)
    wc[:, 0:32, :] = jnp.zeros((4, 32, 3584), u32)

    def ln_block(g):
        cols = pl.ds(pl.multiple_of(g * 128, 128), 128)
        xb = xv[:, cols].astype(f32)
        m = jnp.mean(xb, axis=0, keepdims=True)
        xc = xb - m
        v = jnp.mean(xc * xc, axis=0, keepdims=True)
        xn = xc * jax.lax.rsqrt(v + 1e-5)
        xn = jnp.concatenate([jnp.zeros((64, 128), f32), xn], axis=0).astype(bf16)
        xnt[:, cols] = xn
        xn32[cols, :] = xn.T.astype(f32)

    def stage(src, dst, d0, nd):
        for r in range(0, nd, 56):
            u = pltpu.bitcast(src[16 * (d0 + r):16 * (d0 + r + 56), :], u32)
            for dd in range(56):
                pos = ((r + dd) % 2) * (nd // 2) + (r + dd) // 2
                for half in range(2):
                    dst[half, pl.ds(pos, 8, stride=nd + 2), :] = u[8 * dd:8 * dd + 8, 128 * half:128 * half + 128]

    def pair_rows(st, j, nd):
        return jnp.concatenate([st[half, pl.ds(j * (nd + 2), nd), :] for half in range(2)], axis=1)

    def lhs_heads(st, j, nd):
        u = pair_rows(st, j, nd)
        return pltpu.bitcast(u << 16, f32), pltpu.bitcast(u & u32(0xffff0000), f32)

    def pack_rows(r):
        n = r.shape[0] // 2
        return pltpu.bitcast(pltpu.pack_elementwise([r[:n], r[n:]], packed_dtype=bf16), u32)

    def w1_block(c):
        blk = w1v[:, c * 128:(c + 1) * 128]
        blk = jnp.concatenate([jnp.zeros((64, 128), bf16), blk], axis=0)
        w1t[c * 64:(c + 1) * 64, :] = pltpu.bitcast(blk.T, u32)

    KS = 258

    def make_kde(t):
        cp_k[t].wait()
        if t == 0:
            for half in range(2):
                for h in range(H):
                    kde[half, pl.ds(h * KS, 32), :] = jnp.zeros((32, 128), u32)
        for r in range(KR[t], KR[t + 1], 32):
            u = pltpu.bitcast(wkv[16 * r:16 * (r + 32), :], u32)
            for s_ in range(16):
                a, b_ = u[16 * s_:16 * s_ + 8], u[16 * s_ + 8:16 * s_ + 16]
                lo = (a & u32(0xffff)) | (b_ << 16)
                hi = (a >> 16) | (b_ & u32(0xffff0000))
                row = 32 + r // 2 + s_
                for half in range(2):
                    kde[half, pl.ds(row, 8, stride=2 * KS), :] = lo[:, 128 * half:128 * half + 128]
                    kde[half, pl.ds(row + KS, 8, stride=2 * KS), :] = hi[:, 128 * half:128 * half + 128]

    def kde_tile(h, t):
        return _bf(jnp.concatenate([kde[half, pl.ds(h * KS + 64 * t, 64), :] for half in range(2)], axis=1))

    def chunk_ref(st, c):
        return st.at[:, pl.ds(c * 8 * 114, 8 * 114), :]

    def b_block(c, g, mid=None):
        for j in (2 * g, 2 * g + 1):
            if mid is not None and j == 2 * g + 1:
                mid()
            vs = lhs_heads(chunk_ref(stk, c), j, 112)
            for b in range(2):
                h = 2 * j + b
                wo = jnp.concatenate([wov[h], jnp.zeros((64, E), bf16)], axis=0)
                col = (h % 4) * 896
                wc[h // 4, 32 + 56 * c:32 + 56 * (c + 1), col:col + 512] = pack_rows(_dot_ntm(vs[b], wo))

    def a_block(c, t, mid=None):
        for j in range(8):
            if mid is not None and j == MIDJ:
                mid()
            qs = lhs_heads(chunk_ref(stq, c), j, 112)
            for b in range(2):
                h = 2 * j + b
                a_sh = pack_rows(_dot_ntm(qs[b], kde_tile(h, t)))
                rows = slice(32 + 56 * c, 32 + 56 * (c + 1))
                col = (h % 4) * 896 + 384 + 128 * t
                if t == 0:
                    a_sh = a_sh | wc[h // 4, rows, col:col + 128]
                wc[h // 4, rows, col:col + 128] = a_sh

    def get_v(c):
        cp_v[c].wait()
        stage(wvv, chunk_ref(stk, c), 112 * c, 112)

    def get_q(c):
        cp_q[c].wait()
        stage(wqv, chunk_ref(stq, c), 112 * c, 112)

    for n in range(4):
        get_v(n)
        for g in range(n):
            b_block(n, g)
        cp_o[n].wait()
        for c in range(n + 1):
            mid = None
            if n == 3 and c == 0:
                mid = lambda: get_q(0)
            if n == 3 and c == 3:
                mid = lambda: (make_kde(0), make_kde(1))
            b_block(c, n, mid)

    a_block(0, 0)
    a_block(0, 1, lambda: get_q(1))
    a_block(1, 0)
    a_block(1, 1, lambda: make_kde(2))
    a_block(0, 2)
    a_block(1, 2, lambda: get_q(2))
    a_block(2, 0)
    a_block(2, 1)
    a_block(2, 2, lambda: make_kde(3))
    a_block(0, 3)
    a_block(1, 3, lambda: get_q(3))
    a_block(2, 3, lambda: (cp_x[0].wait(), ln_block(0)))
    a_block(3, 0)
    a_block(3, 1, lambda: (cp_1[0].wait(), cp_1[1].wait()))
    a_block(3, 2, lambda: [w1_block(blk) for blk in range(0, 7)])
    a_block(3, 3, lambda: [w1_block(blk) for blk in range(7, 14)])

    ots[...] = jnp.zeros(ots.shape, ots.dtype)
    cp_2.wait()

    cp_m.wait()
    mem0 = memv[...].astype(f32)
    mem0 = jnp.concatenate([jnp.zeros((8, 64), f32), mem0], axis=1)

    lane = jax.lax.broadcasted_iota(i32, (8, 128), 1)
    lane32 = jax.lax.broadcasted_iota(i32, (32, 128), 1)

    def softmax(sc, mask):
        sc = jnp.where(mask, sc * (E ** -0.5), -1e9)
        mx = jnp.max(sc, axis=0, keepdims=True)
        e = jnp.exp(sc - mx)
        l = jnp.sum(e, axis=0, keepdims=True)
        return e * (1.0 / l)

    def seg_step(g, i, mem_sh, ffn, hook=None):
        xr = xn32[pl.ds(pl.multiple_of(g * 128 + i * 32, 32), 32), :]
        h40 = jnp.concatenate([mem_sh, xr], axis=0)

        def wcol(h, lo, hi):
            return _bf(wc[h // 4, :, (h % 4) * 896 + lo:(h % 4) * 896 + hi])

        m0 = msk[0] != 0
        m1 = msk[1] != 0
        T = [None] * H
        Y = [None] * H
        P = [None] * 5
        box = {}

        def sdot(tb):
            return _dotm(h40, _T(tb))

        def ffn_op(kind, p):
            f0 = POFF[p]
            if kind == 'F':
                hpre = _dot(_bf(w1t[f0 // 2:(f0 + PARTS[p]) // 2, :]), xnt[:, pl.ds(pl.multiple_of(g * 128, 128), 128)])
                ffn['h', p] = (hpre * jax.nn.sigmoid(hpre)).astype(bf16)
            else:
                ns = {512: GSPLIT, 256: 2}.get(PARTS[p], 4)
                rs = D // ns
                o = jnp.concatenate([_dot(w2v[r * rs:(r + 1) * rs, f0:f0 + PARTS[p]], ffn['h', p]) for r in range(ns)], axis=0)
                ffn['o'] = ffn['o'] + o if 'o' in ffn else o

        def do(op):
            kind, a = op[0], int(op[1:], 16) if len(op) > 1 else 0
            if kind == 'T':
                for h in range(4 * a, 4 * a + 4):
                    T[h] = _dotm(h40, wcol(h, 384, 896))
            elif kind == 'Y':
                for h in range(4 * a, 4 * a + 4):
                    Y[h] = jnp.concatenate([_dotm(h40, wcol(h, 0, 384)), T[h][:, :128]], axis=1)
            elif kind == 'S':
                if a < 4:
                    tc = jnp.concatenate([T[4 * a + b][0:32] for b in range(4)], axis=0).astype(bf16)
                    P[a] = softmax(sdot(tc), m0)
                else:
                    tc = jnp.concatenate([T[h][32:40] for h in range(H)], axis=0).astype(bf16)
                    P[4] = softmax(sdot(tc), m1)
            elif kind in 'ab':
                for fop in FSCHED[i].split(',')[0 if kind == 'a' else 1].split('+'):
                    if fop:
                        ffn_op(fop[0], int(fop[1]))
            elif kind == 'L':
                if i == LSTEP:
                    ln_block(jnp.minimum(g + 1, NG - 1))
            elif kind == 'P':
                box['R'] = do_py()

        def do_py():
            m1t = jnp.concatenate([P[a][0:32] for a in range(4)], axis=0).T
            m3 = jnp.concatenate([jnp.where(lane // 32 == b, P[a][32:40], 0.0)
                                  for a in range(4) for b in range(4)], axis=0)
            m3t = m3.T
            m3t = (m3t[0:32] + m3t[32:64]) + (m3t[64:96] + m3t[96:128])
            m4 = jnp.concatenate([jnp.where(lane32 // 32 == a, P[4][0:32], 0.0) for a in range(4)], axis=0)
            m4t = m4.T
            m5 = jnp.concatenate([jnp.where(lane // 8 == hh, P[4][32:40], 0.0) for hh in range(16)], axis=0)
            m5t = m5.T
            w = m5t[0:8]
            for r in range(1, 16):
                w = w + m5t[8 * r:8 * r + 8]
            pcat = []
            for gg in range(4):
                third = m4t[8 * gg:8 * gg + 8]
                for a in range(1, 4):
                    third = third + m4t[8 * (4 * a + gg):8 * (4 * a + gg) + 8]
                pcat.append(jnp.concatenate([m1t[32 * gg:32 * gg + 32], third], axis=0))
            pcat.append(jnp.concatenate([m3t, w], axis=0))
            pcat = jnp.concatenate(pcat, axis=1)
            ycat = [jnp.concatenate([Y[4 * a + gg][0:32] for a in range(4)], axis=0).astype(bf16) for gg in range(4)]
            ycat.append(jnp.concatenate([Y[h][32:40] for h in range(H)], axis=0).astype(bf16))
            ycat = jnp.concatenate(ycat, axis=0)
            return _dotm(pcat, ycat)

        for op in ORDER.split():
            if op == 'O':
                if hook is not None:
                    hook()
            else:
                do(op)
        R = box['R']
        res = R[8:40]
        mem_next = jnp.concatenate([jnp.zeros((8, 64), f32), R[0:8, :D]], axis=1)
        return mem_next, res

    def out_copy(g):
        cols = pl.ds(pl.multiple_of(g * 128, 128), 128)
        return pltpu.make_async_copy(ob.at[:, cols], o_h.at[:, cols], osem.at[0])

    def flush(g, ffn_t):
        cols = pl.ds(pl.multiple_of(g * 128, 128), 128)
        rt = rb[...].T
        ob[:, cols] = (xv[:, cols].astype(f32) + (rt[:D] + ffn_t)).astype(ob.dtype)

    rb[...] = jnp.zeros(rb.shape, rb.dtype)

    def body(g, mem_sh):
        gp = jnp.maximum(g - 1, 0)
        ffn = {}
        for i in range(4):
            hook = (lambda: flush(gp, ots[...])) if i == 0 else None
            mem_sh, r = seg_step(g, i, mem_sh, ffn, hook)
            rb[i * 32:(i + 1) * 32, :] = r
        ots[...] = ffn['o']

        @pl.when(g > 0)
        def _():
            out_copy(g - 1).start()

        @pl.when(g == 0)
        def _():
            cp_x[1].wait()
        return mem_sh

    jax.lax.fori_loop(0, NGRUN, body, mem0)
    flush(NGRUN - 1, ots[...])
    out_copy(NGRUN - 1).start()
    for g_ in range(NGRUN):
        out_copy(g_).wait()


@jax.jit
def pallas_parallel_sum__memory_aug_recurrent_mem_tr__dense_activation_silu__prompt_kernel(
    A_x,
    A_mem0,
    A_Wq,
    A_Wk,
    A_Wv,
    A_Wo,
    A_seg_len,
    B_x,
    B_w1,
    B_w2,
):
    dt = A_x.dtype
    any_spec = pl.BlockSpec(memory_space=pl.ANY)
    out = pl.pallas_call(
        kernel,
        out_shape=jax.ShapeDtypeStruct((D, S), dt),
        in_specs=[any_spec] * 8,
        out_specs=any_spec,
        scratch_shapes=[
            pltpu.VMEM((D, S), dt),
            pltpu.VMEM((8, D), dt),
            pltpu.VMEM((D * H, E), dt),
            pltpu.VMEM((D * H, E), dt),
            pltpu.VMEM((D * H, E), dt),
            pltpu.VMEM((H, D, E), dt),
            pltpu.VMEM((D, F), dt),
            pltpu.VMEM((D, F), dt),
            pltpu.VMEM((4, 256, 3584), u32),
            pltpu.VMEM((F // 2, DP), u32),
            pltpu.VMEM((DP, S), dt),
            pltpu.VMEM((D, 128), f32),
            pltpu.VMEM((S, DP), f32),
            pltpu.VMEM((2, 3648, 128), u32),
            pltpu.VMEM((2, 3648, 128), u32),
            pltpu.VMEM((2, H * 258, 128), u32),
            pltpu.VMEM((2, 40, 128), i32),
            pltpu.VMEM((D, S), dt),
            pltpu.VMEM((128, DP), f32),
            pltpu.SemaphoreType.DMA((NSEM,)),
            pltpu.SemaphoreType.DMA((1,)),
        ],
        compiler_params=pltpu.CompilerParams(vmem_limit_bytes=110 * 1024 * 1024),
    )(A_x.reshape(S, D).T, A_mem0.reshape(8, D), A_Wq.reshape(D * H, E), A_Wk.reshape(D * H, E),
      A_Wv.reshape(D * H, E), jnp.transpose(A_Wo, (0, 2, 1)), B_w1, B_w2.T)
    return out.T.reshape(1, S, D)
```

```python
import jax
import jax.numpy as jnp
from jax.experimental import pallas as pl
from jax.experimental.pallas import tpu as pltpu

D = 448
DP = 512
H = 16
E = 256
F = 1792
S = 2048
NG = S // 128
KS = 258
KR = (0, 64, 192, 320, 448)
PARTS = (512, 384, 512, 384)
POFF = (0, 512, 896, 1408)
FSPLIT = (2, 4, 2, 4)
FSCHED = (("F0", "F1"), ("F2", "G0"), ("G1", "F3"), ("G2", "G3"))
u32, i32, f32, bf16 = jnp.uint32, jnp.int32, jnp.float32, jnp.bfloat16


def _bf(x):
    return pltpu.bitcast(x, bf16)


def _T(x):
    return _bf(pltpu.bitcast(x.T, u32))


def _dot(a, b):
    return jax.lax.dot_general(a, b, (((1,), (0,)), ((), ())), preferred_element_type=f32)


def _dot_nt(a, b):
    return jax.lax.dot_general(a, b, (((1,), (1,)), ((), ())), preferred_element_type=f32)


def _kernel(x_h, mem_h, wq_h, wk_h, wv_h, wo_h, w1_h, w2_h, o_h,
            xv, memv, wqv, wkv, wvv, wov, w1v, w2v,
            wc, w1t, xnt, xn32, ots, stq, stv, kde, msk, ob, rb, sem, osem):
    def cp(src, dst, k):
        return pltpu.make_async_copy(src, dst, sem.at[k])

    QR = D * H // 4
    cp_m = cp(mem_h, memv, 0)
    cp_v = [cp(wv_h.at[pl.ds(QR * c, QR)], wvv.at[pl.ds(QR * c, QR)], 1 + c) for c in range(4)]
    cp_o = [cp(wo_h.at[pl.ds(4 * g, 4)], wov.at[pl.ds(4 * g, 4)], 5 + g) for g in range(4)]
    cp_q = [cp(wq_h.at[pl.ds(QR * c, QR)], wqv.at[pl.ds(QR * c, QR)], 9 + c) for c in range(4)]
    cp_k = [cp(wk_h.at[pl.ds(16 * KR[t], 16 * (KR[t + 1] - KR[t]))],
               wkv.at[pl.ds(16 * KR[t], 16 * (KR[t + 1] - KR[t]))], 13 + t) for t in range(4)]
    cp_x = [cp(x_h.at[:, pl.ds(0, 256)], xv.at[:, pl.ds(0, 256)], 17),
            cp(x_h.at[:, pl.ds(256, S - 256)], xv.at[:, pl.ds(256, S - 256)], 18)]
    cp_1 = [cp(w1_h.at[:, pl.ds(896 * c, 896)], w1v.at[:, pl.ds(896 * c, 896)], 19 + c) for c in range(2)]
    cp_2 = cp(w2_h, w2v, 21)
    order = [cp_m]
    for c in range(4):
        order += [cp_v[c], cp_o[c]]
    order += [cp_q[0], cp_k[0], cp_k[1], cp_q[1], cp_k[2], cp_q[2], cp_k[3], cp_q[3],
              cp_x[0], cp_1[0], cp_1[1], cp_2, cp_x[1]]
    for c_ in order:
        c_.start()

    k_i = jax.lax.broadcasted_iota(i32, (40, 128), 0)
    l_i = jax.lax.broadcasted_iota(i32, (40, 128), 1)
    q_i = l_i % 32
    msk[0] = ((q_i < 8) | (k_i <= q_i)).astype(i32)
    msk[1] = (k_i <= 32 + l_i % 8).astype(i32)
    wc[:, 0:32, :] = jnp.zeros((4, 32, 3584), u32)

    def ln_block(g):
        cols = pl.ds(pl.multiple_of(g * 128, 128), 128)
        xb = xv[:, cols].astype(f32)
        m = jnp.mean(xb, axis=0, keepdims=True)
        xc = xb - m
        v = jnp.mean(xc * xc, axis=0, keepdims=True)
        xn = xc * jax.lax.rsqrt(v + 1e-5)
        xn = jnp.concatenate([jnp.zeros((64, 128), f32), xn], axis=0).astype(bf16)
        xnt[:, cols] = xn
        xn32[cols, :] = xn.T.astype(f32)

    def w1_block(c):
        blk = w1v[:, c * 128:(c + 1) * 128]
        blk = jnp.concatenate([jnp.zeros((64, 128), bf16), blk], axis=0)
        w1t[c * 64:(c + 1) * 64, :] = pltpu.bitcast(blk.T, u32)

    def stage(src, dst, d0, nd):
        for r in range(0, nd, 56):
            u = pltpu.bitcast(src[16 * (d0 + r):16 * (d0 + r + 56), :], u32)
            for dd in range(56):
                pos = ((r + dd) % 2) * (nd // 2) + (r + dd) // 2
                for half in range(2):
                    dst[half, pl.ds(pos, 8, stride=nd + 2), :] = u[8 * dd:8 * dd + 8, 128 * half:128 * half + 128]

    def chunk_ref(st, c):
        return st.at[:, pl.ds(c * 8 * 114, 8 * 114), :]

    def lhs_heads(st, j, nd):
        u = jnp.concatenate([st[half, pl.ds(j * (nd + 2), nd), :] for half in range(2)], axis=1)
        return pltpu.bitcast(u << 16, f32), pltpu.bitcast(u & u32(0xffff0000), f32)

    def pack_rows(r):
        n = r.shape[0] // 2
        return pltpu.bitcast(pltpu.pack_elementwise([r[:n], r[n:]], packed_dtype=bf16), u32)

    def make_kde(t):
        cp_k[t].wait()
        if t == 0:
            for half in range(2):
                for h in range(H):
                    kde[half, pl.ds(h * KS, 32), :] = jnp.zeros((32, 128), u32)
        for r in range(KR[t], KR[t + 1], 32):
            u = pltpu.bitcast(wkv[16 * r:16 * (r + 32), :], u32)
            for s_ in range(16):
                a, b_ = u[16 * s_:16 * s_ + 8], u[16 * s_ + 8:16 * s_ + 16]
                lo = (a & u32(0xffff)) | (b_ << 16)
                hi = (a >> 16) | (b_ & u32(0xffff0000))
                row = 32 + r // 2 + s_
                for half in range(2):
                    kde[half, pl.ds(row, 8, stride=2 * KS), :] = lo[:, 128 * half:128 * half + 128]
                    kde[half, pl.ds(row + KS, 8, stride=2 * KS), :] = hi[:, 128 * half:128 * half + 128]

    def kde_tile(h, t):
        return _bf(jnp.concatenate([kde[half, pl.ds(h * KS + 64 * t, 64), :] for half in range(2)], axis=1))

    def b_block(c, g, mid=None):
        for j in (2 * g, 2 * g + 1):
            if mid is not None and j == 2 * g + 1:
                mid()
            vs = lhs_heads(chunk_ref(stv, c), j, 112)
            for b in range(2):
                h = 2 * j + b
                wo = jnp.concatenate([wov[h], jnp.zeros((64, E), bf16)], axis=0)
                col = (h % 4) * 896
                wc[h // 4, 32 + 56 * c:32 + 56 * (c + 1), col:col + 512] = pack_rows(_dot_nt(vs[b], wo))

    def a_block(c, t, mid=None):
        for j in range(8):
            if mid is not None and j == 6:
                mid()
            qs = lhs_heads(chunk_ref(stq, c), j, 112)
            for b in range(2):
                h = 2 * j + b
                a_sh = pack_rows(_dot_nt(qs[b], kde_tile(h, t)))
                rows = slice(32 + 56 * c, 32 + 56 * (c + 1))
                col = (h % 4) * 896 + 384 + 128 * t
                if t == 0:
                    a_sh = a_sh | wc[h // 4, rows, col:col + 128]
                wc[h // 4, rows, col:col + 128] = a_sh

    def get_v(c):
        cp_v[c].wait()
        stage(wvv, chunk_ref(stv, c), 112 * c, 112)

    def get_q(c):
        cp_q[c].wait()
        stage(wqv, chunk_ref(stq, c), 112 * c, 112)

    for n in range(4):
        get_v(n)
        for g in range(n):
            b_block(n, g, (lambda: (cp_o[3].wait(), get_q(0))) if (n, g) == (3, 2) else None)
        if n < 3:
            cp_o[n].wait()
        for c in range(n + 1):
            b_block(c, n, (lambda: (make_kde(0), make_kde(1))) if (n, c) == (3, 3) else None)
    a_block(0, 0)
    a_block(0, 1, lambda: get_q(1))
    a_block(1, 0)
    a_block(1, 1, lambda: make_kde(2))
    a_block(0, 2)
    a_block(1, 2, lambda: get_q(2))
    a_block(2, 0)
    a_block(2, 1)
    a_block(2, 2, lambda: (cp_q[3].wait(), cp_x[0].wait(), make_kde(3)))
    a_block(0, 3, lambda: stage(wqv, chunk_ref(stq, 3), 336, 112))
    a_block(1, 3, lambda: ln_block(0))
    a_block(2, 3)
    a_block(3, 0, lambda: (cp_1[0].wait(), cp_1[1].wait()))
    a_block(3, 1, lambda: [w1_block(blk) for blk in range(0, 5)])
    a_block(3, 2, lambda: [w1_block(blk) for blk in range(5, 10)])
    a_block(3, 3, lambda: [w1_block(blk) for blk in range(10, 14)])

    ots[...] = jnp.zeros(ots.shape, ots.dtype)
    cp_2.wait()
    cp_m.wait()
    mem0 = jnp.concatenate([jnp.zeros((8, 64), f32), memv[...].astype(f32)], axis=1)

    lane = jax.lax.broadcasted_iota(i32, (8, 128), 1)
    lane32 = jax.lax.broadcasted_iota(i32, (32, 128), 1)

    def softmax(sc, mask):
        sc = jnp.where(mask, sc * (E ** -0.5), -1e9)
        mx = jnp.max(sc, axis=0, keepdims=True)
        e = jnp.exp(sc - mx)
        l = jnp.sum(e, axis=0, keepdims=True)
        return e * (1.0 / l)

    def seg_step(g, i, mem_sh, ffn, hook):
        xr = xn32[pl.ds(pl.multiple_of(g * 128 + i * 32, 32), 32), :]
        t40 = jnp.concatenate([mem_sh, xr], axis=0)
        m0 = msk[0] != 0
        m1 = msk[1] != 0
        T, Y, P = [None] * H, [None] * H, [None] * 5

        def wcol(h, lo, hi):
            return _bf(wc[h // 4, :, (h % 4) * 896 + lo:(h % 4) * 896 + hi])

        def t_part(a):
            for h in range(4 * a, 4 * a + 4):
                T[h] = _dot(t40, wcol(h, 384, 896))

        def y_part(a):
            for h in range(4 * a, 4 * a + 4):
                Y[h] = jnp.concatenate([_dot(t40, wcol(h, 0, 384)), T[h][:, :128]], axis=1)

        def scores(a):
            if a < 4:
                tc = jnp.concatenate([T[4 * a + b][0:32] for b in range(4)], axis=0).astype(bf16)
            else:
                tc = jnp.concatenate([T[h][32:40] for h in range(H)], axis=0).astype(bf16)
            P[a] = softmax(_dot(t40, _T(tc)), m0 if a < 4 else m1)

        def ffn_op(op):
            p = int(op[1])
            f0 = POFF[p]
            if op[0] == 'F':
                hpre = _dot(_bf(w1t[f0 // 2:(f0 + PARTS[p]) // 2, :]),
                            xnt[:, pl.ds(pl.multiple_of(g * 128, 128), 128)])
                ffn['h', p] = (hpre * jax.nn.sigmoid(hpre)).astype(bf16)
            else:
                rs = D // FSPLIT[p]
                o = jnp.concatenate([_dot(w2v[r * rs:(r + 1) * rs, f0:f0 + PARTS[p]], ffn['h', p])
                                     for r in range(FSPLIT[p])], axis=0)
                ffn['o'] = ffn['o'] + o if 'o' in ffn else o

        def py():
            m1t = jnp.concatenate([P[a][0:32] for a in range(4)], axis=0).T
            m3 = jnp.concatenate([jnp.where(lane // 32 == b, P[a][32:40], 0.0)
                                  for a in range(4) for b in range(4)], axis=0)
            m3t = m3.T
            m3t = (m3t[0:32] + m3t[32:64]) + (m3t[64:96] + m3t[96:128])
            m4 = jnp.concatenate([jnp.where(lane32 // 32 == a, P[4][0:32], 0.0) for a in range(4)], axis=0)
            m4t = m4.T
            m5 = jnp.concatenate([jnp.where(lane // 8 == hh, P[4][32:40], 0.0) for hh in range(16)], axis=0)
            m5t = m5.T
            w = m5t[0:8]
            for r in range(1, 16):
                w = w + m5t[8 * r:8 * r + 8]
            pcat = []
            for gg in range(4):
                third = m4t[8 * gg:8 * gg + 8]
                for a in range(1, 4):
                    third = third + m4t[8 * (4 * a + gg):8 * (4 * a + gg) + 8]
                pcat.append(jnp.concatenate([m1t[32 * gg:32 * gg + 32], third], axis=0))
            pcat.append(jnp.concatenate([m3t, w], axis=0))
            pcat = jnp.concatenate(pcat, axis=1)
            ycat = [jnp.concatenate([Y[4 * a + gg][0:32] for a in range(4)], axis=0).astype(bf16)
                    for gg in range(4)]
            ycat.append(jnp.concatenate([Y[h][32:40] for h in range(H)], axis=0).astype(bf16))
            return _dot(pcat, jnp.concatenate(ycat, axis=0))

        t_part(0)
        if hook is not None:
            hook()
        t_part(1)
        t_part(2)
        t_part(3)
        y_part(0)
        for a in range(5):
            scores(a)
        y_part(1)
        y_part(2)
        y_part(3)
        ffn_op(FSCHED[i][0])
        if i == 3:
            ln_block(jnp.minimum(g + 1, NG - 1))
        R = py()
        ffn_op(FSCHED[i][1])
        mem_next = jnp.concatenate([jnp.zeros((8, 64), f32), R[0:8, :D]], axis=1)
        return mem_next, R[8:40]

    def out_copy(g):
        cols = pl.ds(pl.multiple_of(g * 128, 128), 128)
        return pltpu.make_async_copy(ob.at[:, cols], o_h.at[:, cols], osem.at[0])

    def flush(g):
        cols = pl.ds(pl.multiple_of(g * 128, 128), 128)
        rt = rb[...].T
        ob[:, cols] = (xv[:, cols].astype(f32) + (rt[:D] + ots[...])).astype(ob.dtype)

    rb[...] = jnp.zeros(rb.shape, rb.dtype)

    def body(g, mem_sh):
        gp = jnp.maximum(g - 1, 0)
        ffn = {}
        for i in range(4):
            mem_sh, r = seg_step(g, i, mem_sh, ffn, (lambda: flush(gp)) if i == 0 else None)
            rb[i * 32:(i + 1) * 32, :] = r
        ots[...] = ffn['o']

        @pl.when(g > 0)
        def _():
            out_copy(g - 1).start()

        @pl.when(g == 0)
        def _():
            cp_x[1].wait()
        return mem_sh

    jax.lax.fori_loop(0, NG, body, mem0)
    flush(NG - 1)
    out_copy(NG - 1).start()
    for g_ in range(NG):
        out_copy(g_).wait()


@jax.jit
def pallas_parallel_sum__memory_aug_recurrent_mem_tr__dense_activation_silu__prompt_kernel(
    A_x,
    A_mem0,
    A_Wq,
    A_Wk,
    A_Wv,
    A_Wo,
    A_seg_len,
    B_x,
    B_w1,
    B_w2,
):
    del A_seg_len, B_x
    dt = A_x.dtype
    hbm = pl.BlockSpec(memory_space=pl.ANY)
    out = pl.pallas_call(
        _kernel,
        out_shape=jax.ShapeDtypeStruct((D, S), dt),
        in_specs=[hbm] * 8,
        out_specs=hbm,
        scratch_shapes=[
            pltpu.VMEM((D, S), dt),
            pltpu.VMEM((8, D), dt),
            pltpu.VMEM((D * H, E), dt),
            pltpu.VMEM((D * H, E), dt),
            pltpu.VMEM((D * H, E), dt),
            pltpu.VMEM((H, D, E), dt),
            pltpu.VMEM((D, F), dt),
            pltpu.VMEM((D, F), dt),
            pltpu.VMEM((4, 256, 3584), u32),
            pltpu.VMEM((F // 2, DP), u32),
            pltpu.VMEM((DP, S), dt),
            pltpu.VMEM((S, DP), f32),
            pltpu.VMEM((D, 128), f32),
            pltpu.VMEM((2, 3648, 128), u32),
            pltpu.VMEM((2, 3648, 128), u32),
            pltpu.VMEM((2, H * KS, 128), u32),
            pltpu.VMEM((2, 40, 128), i32),
            pltpu.VMEM((D, S), dt),
            pltpu.VMEM((128, DP), f32),
            pltpu.SemaphoreType.DMA((22,)),
            pltpu.SemaphoreType.DMA((1,)),
        ],
        compiler_params=pltpu.CompilerParams(vmem_limit_bytes=110 * 1024 * 1024),
    )(A_x.reshape(S, D).T, A_mem0.reshape(8, D), A_Wq.reshape(D * H, E), A_Wk.reshape(D * H, E),
      A_Wv.reshape(D * H, E), jnp.transpose(A_Wo, (0, 2, 1)), B_w1, B_w2.T)
    return out.T.reshape(1, S, D)
```
